```python
import os as _os
_os.environ.setdefault("JAX_PLATFORMS", "cpu")
import jax
import jax.numpy as jnp

def _softmax(x, axis=-1):
    return jax.nn.softmax(x, axis=axis)
def _gelu(x):
    return jax.nn.gelu(x, approximate=True)
def _silu(x):
    return jax.nn.silu(x)
def _sigmoid(x):
    return jax.nn.sigmoid(x)
def _layernorm(x, axis=-1, eps=1e-5):
    m = jnp.mean(x, axis=axis, keepdims=True)
    v = jnp.var(x, axis=axis, keepdims=True)
    return (x - m) / jnp.sqrt(v + eps)
def _scatter_add(tgt, idx, src, axis=0):
    return tgt.at[idx].add(src)
def _segment_sum(src, seg, n):
    return jax.ops.segment_sum(src, seg, n)
class _Rng:
    def __init__(self, key):
        self._k = key
    def _next(self):
        self._k, sub = jax.random.split(self._k)
        return sub
    def normal(self, shape):
        return jax.random.normal(self._next(), shape, dtype=jnp.bfloat16)
    def randint(self, lo, hi, shape):
        return jax.random.randint(self._next(), shape, lo, hi, dtype=jnp.int32)
    def uniform(self, shape, lo=0.0, hi=1.0):
        return jax.random.uniform(self._next(), shape, jnp.bfloat16, lo, hi)
    def permutation(self, n):
        return jax.random.permutation(self._next(), n)


kernel_name = 'recurrent_scan__spectral_gfnet__swiglu_ffn__prompt'

def setup_inputs():
    _rng = _Rng(jax.random.key(int.from_bytes(__import__("os").urandom(4), "little")))
    _w = (lambda a: (lambda t: t.astype(jnp.bfloat16) if jnp.issubdtype(t.dtype, jnp.floating) else t)(jnp.asarray(a)))
    def _A_setup():
        B, S, D = 1, 2048, 640
        Df = D // 2 + 1
        return {
            "x": _w((lambda *s: _rng.normal(s) * 0.05)(B, S, D)),
            "w_r": _w((lambda *s: _rng.normal(s) * 0.05)(S, Df) * 0.02),
            "w_i": _w((lambda *s: _rng.normal(s) * 0.05)(S, Df) * 0.02),
        }
    _A_in = _A_setup()

    def _B_setup():
        B, S, D, F = 1, 2048, 640, 1536
        return {
            "x": _w((lambda *s: _rng.normal(s) * 0.05)(B, S, D)),
            "w_gate": _w((lambda *s: _rng.normal(s) * 0.05)(D, F)),
            "w_up": _w((lambda *s: _rng.normal(s) * 0.05)(D, F)),
            "w_down": _w((lambda *s: _rng.normal(s) * 0.05)(F, D)),
        }
    _B_in = _B_setup()

    return {
        "A_x": _A_in["x"],
        "A_w_r": _A_in["w_r"],
        "A_w_i": _A_in["w_i"],
        "B_x": _B_in["x"],
        "B_w_gate": _B_in["w_gate"],
        "B_w_up": _B_in["w_up"],
        "B_w_down": _B_in["w_down"],
    }

def reference(A_x, A_w_r, A_w_i, B_x, B_w_gate, B_w_up, B_w_down):
    def _A_ref(x, w_r, w_i):
        B, S, D = x.shape
        X = (lambda x, axes=(-2,-1): jnp.fft.rfft2(x.astype(jnp.float32), axes=axes))(x, axes=(-2, -1))
        W = w_r + 1j * w_i
        X = X * W
        y = (lambda x, s, axes=(-2,-1): jnp.fft.irfft2(x, s=s, axes=axes).astype(jnp.bfloat16))(X, (S, D), axes=(-2, -1))
        return y

    def _B_ref(x, w_gate, w_up, w_down):
        g = _silu(x @ w_gate)
        u = x @ w_up
        return (g * u) @ w_down

    x = A_x
    xn = _layernorm(x, axis=-1)
    s = _A_ref(xn, A_w_r, A_w_i)
    g = _silu(_B_ref(xn, B_w_gate, B_w_up, B_w_down))
    return x + s * g
```

```python
import functools
import math

import numpy as np
import jax
import jax.numpy as jnp
import jax.experimental.pallas as pl
import jax.experimental.pallas.tpu as pltpu

S, D, F = 2048, 640, 1536
DF = D // 2 + 1
TM = 256
NT = S // TM
NC = 6
FC = F // NC
UNROLL = 2
LN_LAG = 4
DFT_AT = (3, 5, 7)
NA, NB = 32, 64
EPS = 1e-5


def _freq_of_lane():
    l = np.arange(128)
    ka = np.where(l < 64, 1 + 5 * l, 4 + 5 * (l - 64))
    kb = np.where(l < 64, 2 + 5 * l, 3 + 5 * (l - 64))
    kc = np.where(l <= 64, 5 * l, -1)
    return ka, kb, kc


def _constants():
    ka, kb, kc = _freq_of_lane()
    n2 = np.arange(128)[:, None]
    sig = np.where(np.arange(128) < 64, 1.0, -1.0)[None, :]

    def pair(k):
        th = 2 * np.pi * ((n2 * k[None, :]) % D) / D
        c, s = np.cos(th), np.sin(th)
        return np.block([[c, -s], [sig * s, sig * c]])

    fa, fb = pair(ka), pair(kb)
    valid = (kc >= 0)[None, :]
    th = 2 * np.pi * ((n2 * np.maximum(kc, 0)[None, :]) % D) / D
    fc = np.concatenate([np.cos(th) * valid, -np.sin(th) * valid], axis=1)
    alpha = np.where((kc == 0) | (kc == D // 2), 1.0, 2.0)
    alpha2 = np.concatenate([alpha, alpha])[:, None]
    dfwd = np.concatenate([fa, fb, fc], axis=0)
    dinv = np.concatenate([fa.T * (2.0 / D), fb.T * (2.0 / D)], axis=0)
    dinvc = fc.T * alpha2 / D

    b = np.arange(NB)[None, None, :]
    d = np.arange(NB)[None, :, None]
    c = np.arange(NA)[:, None, None]
    ph = 2 * np.pi * ((b * (c + NA * d)) % S) / S
    mr, mi = np.cos(ph), -np.sin(ph)
    sf = np.concatenate([np.concatenate([mr, -mi], axis=2),
                         np.concatenate([mi, mr], axis=2)], axis=1)
    si = np.transpose(sf, (0, 2, 1)) / S

    ang = 2 * np.pi * (np.arange(4)[:, None] * np.arange(8)[None, :]).reshape(-1) / NA
    tw = np.stack([np.cos(ang), np.sin(ang)]).astype(np.float32)
    bf = jnp.bfloat16

    def pairs(a):
        u = a.astype(bf).view(np.uint16).astype(np.uint32)
        return u[..., 0::2, :] | (u[..., 1::2, :] << 16)

    return tw, tuple(pairs(a) for a in (dfwd, dinv, dinvc, sf, si))


def _cmul_const(z, k, n, sign):
    re, im = z
    k = k % n
    if k == 0:
        return z
    c = math.cos(2 * math.pi * k / n)
    s = sign * math.sin(2 * math.pi * k / n)
    if 8 * k == n:
        return ((re - im) * c, (re + im) * c) if sign > 0 else ((re + im) * c, (im - re) * c)
    if 8 * k == 3 * n:
        return ((re + im) * c, (im - re) * c) if sign > 0 else ((re - im) * c, (re + im) * c)
    return (re * c - im * s, re * s + im * c)


def _fft(load, idx, sign, store=None):
    n = len(idx)
    if n == 1:
        return [load(idx[0])]
    ev = yield from _fft(load, idx[0::2], sign)
    od = yield from _fft(load, idx[1::2], sign)
    out = [None] * n
    for k in range(n // 2):
        er, ei = ev[k]
        if 4 * k == n:
            orr, oi = od[k]
            if sign > 0:
                out[k], out[k + n // 2] = (er - oi, ei + orr), (er + oi, ei - orr)
            else:
                out[k], out[k + n // 2] = (er + oi, ei - orr), (er - oi, ei + orr)
        else:
            tr, ti = _cmul_const(od[k], k, n, sign)
            out[k], out[k + n // 2] = (er + tr, ei + ti), (er - tr, ei - ti)
        if store is not None:
            store(k, out[k])
            store(k + n // 2, out[k + n // 2])
        yield
    return out


def _chain(*gens):
    for g in gens:
        yield from g


def _interleave(mxu, n_mxu, vpu, n_vpu):
    done = 0
    for m in range(n_mxu):
        next(mxu)
        target = (m + 1) * n_vpu // n_mxu
        while done < target:
            next(vpu)
            done += 1
    for _ in vpu:
        pass
    for _ in mxu:
        pass


C1, C2 = math.cos(2 * math.pi / 5), math.cos(4 * math.pi / 5)
S1, S2 = math.sin(2 * math.pi / 5), math.sin(4 * math.pi / 5)


def _mult(v, n):
    return v if isinstance(v, int) else pl.multiple_of(v, n)


def _dot(a, b):
    return jnp.dot(a, b, preferred_element_type=jnp.float32)


def _silu_times(v, u):
    hv = 0.5 * v
    a = hv * u
    return a + a * jnp.tanh(hv)


def _kernel(tw_ref, x_hbm, wr_hbm, wi_hbm, wg_hbm, wu_hbm, wd_hbm,
            dfwd_hbm, dinv_hbm, dinvc_hbm, sf_hbm, si_hbm,
            o_hbm,
            x_v, wr_v, wi_v, wg_v, wu_v, wd_v, dfwd_v, dinv_v, dinvc_v, sf_v, si_v,
            xn_v, h_v, z_v, t_v, u_v, wq_v, wp_v, o_v, sem_x, sem_w, sem_o):
    f32, bf16 = jnp.float32, jnp.bfloat16

    def x_copy(i):
        return pltpu.make_async_copy(x_hbm.at[:, i], x_v.at[i], sem_x.at[i])

    class ColCopy:
        def __init__(self, src, dst, slabs, sem0):
            self.copies = [pltpu.make_async_copy(src.at[:, pl.ds(128 * n, 128)], dst.bitcast(bf16).at[n], sem_w.at[sem0 + n])
                           for n in slabs]

        def start(self):
            for c in self.copies:
                c.start()

        def wait(self):
            for c in self.copies:
                c.wait()

    def wide(ref, slabs, rows=slice(None)):
        v = jnp.concatenate([ref[n, rows, :] for n in slabs], axis=1)
        return v if v.dtype == bf16 else pltpu.bitcast(v, bf16)

    def o_copy(i):
        return pltpu.make_async_copy(o_v.at[i], o_hbm.at[:, i], sem_o.at[i])

    g_copies = [ColCopy(wg_hbm, wg_v, (2 * j, 2 * j + 1), 0) for j in range(NC)]
    u_copies = [ColCopy(wu_hbm, wu_v, (2 * j, 2 * j + 1), 12) for j in range(NC)]
    whole = [pltpu.make_async_copy(s_, d_, sem_w.at[29 + n]) for n, (s_, d_) in enumerate([
        (dfwd_hbm, dfwd_v), (wr_hbm, wr_v), (wi_hbm, wi_v), (sf_hbm, sf_v),
        (si_hbm, si_v), (dinv_hbm, dinv_v), (dinvc_hbm, dinvc_v)])]
    c_dfwd, c_wr, c_wi, c_sf, c_si, c_dinv, c_dinvc = whole
    c_wd = ColCopy(wd_hbm, wd_v, range(5), 24)

    for c in (x_copy(0), g_copies[0], u_copies[0]):
        c.start()

    def tile(i):
        return pl.ds(_mult(i * TM, TM), TM)

    def ptile(i):
        return pl.ds(_mult(i * (TM // 2), TM // 2), TM // 2)

    class Pin:
        def __init__(self, i):
            self.keep = jax.lax.broadcasted_iota(jnp.int32, (8, 128), 0) >= -i
            self.dep = None
            self.queue = [[] for _ in range(5)]

        def mark(self, v):
            self.dep = v[0:8, 0:128]

        def after(self, v):
            if self.dep is None:
                return v
            n = v.shape[0] // 8
            dep = self.dep if v.dtype == f32 else pltpu.bitcast(self.dep, v.dtype)
            return jnp.where(jnp.concatenate([self.keep] * n, axis=0), v, jnp.concatenate([dep] * n, axis=0))

        def due(self, d, lag):
            self.queue[lag].append(d if d.dtype == jnp.uint32 else pltpu.bitcast(d, jnp.uint32))

        def lhs(self, slabs, rows):
            parts = [xn_v[n, rows, :] for n in slabs]
            for n, d in enumerate(self.queue[0]):
                v, r = parts[n % len(parts)], d.shape[0]
                head = jnp.where(jnp.concatenate([self.keep] * (r // 8), axis=0), v[:r], d)
                parts[n % len(parts)] = head if r == v.shape[0] else jnp.concatenate([head, v[r:]], axis=0)
            self.queue = self.queue[1:] + [[]]
            return pltpu.bitcast(jnp.concatenate(parts, axis=1), bf16)

    def gate_up_steps(rows, j, pin):
        xt = pin.lhs([4], rows)
        pair = (2 * j, 2 * j + 1)
        gt, ut = _dot(xt, wide(wg_v, pair, slice(256, D // 2))), _dot(xt, wide(wu_v, pair, slice(256, D // 2)))
        pin.mark(gt)
        yield
        for n in range(2):
            g = _dot(pin.lhs(range(4), rows), wide(wg_v, [pair[n]], slice(0, 256)))
            pin.mark(g)
            g = g + gt[:, 128 * n:128 * (n + 1)]
            yield
            u = _dot(pin.lhs(range(4), rows), wide(wu_v, [pair[n]], slice(0, 256)))
            pin.mark(u)
            h_v[pair[n], rows, :] = pltpu.bitcast(
                _silu_times(g, u + ut[:, 128 * n:128 * (n + 1)]).astype(bf16), jnp.uint32)
            yield

    def pack(re, im):
        return (pltpu.bitcast(re.astype(f32), jnp.uint32)
                | (pltpu.bitcast(im.astype(f32), jnp.uint32) >> 16))

    def layernorm(i, m, pin):
        x = jnp.concatenate(
            [pltpu.bitcast(pin.after(pltpu.bitcast(x_v[i, m, :, 128 * n:128 * (n + 1)], jnp.uint32)), bf16)
             for n in range(5)], axis=1).astype(f32)
        xc = x - jnp.mean(x, axis=-1, keepdims=True)
        v = jnp.mean(xc * xc, axis=-1, keepdims=True)
        xn = pltpu.bitcast((xc * jax.lax.rsqrt(v + EPS)).astype(bf16), jnp.uint32)
        return [xn[:, 128 * n:128 * (n + 1)] for n in range(5)]

    def store_xn(i, m, slabs):
        rows = pl.ds(_mult(i * (TM // 2) + m * (NB // 2), NB // 2), NB // 2)
        for n in range(5):
            xn_v[n, rows, :] = slabs[n]

    def radix4(v, sign):
        re = [v[NB * m:NB * (m + 1), :128] for m in range(4)]
        im = [v[NB * m:NB * (m + 1), 128:] for m in range(4)]
        ar, ai, br, bi = re[0] + re[2], im[0] + im[2], re[0] - re[2], im[0] - im[2]
        cr, ci, dr, di = re[1] + re[3], im[1] + im[3], re[1] - re[3], im[1] - im[3]
        lo, hi = (br + di, bi - dr), (br - di, bi + dr)
        out = [(ar + cr, ai + ci), lo if sign < 0 else hi, (ar - cr, ai - ci), hi if sign < 0 else lo]
        return jnp.concatenate([jnp.concatenate(o, axis=1) for o in out], axis=0)

    def filt(q, lt, pin):
        lanes = pl.ds(_mult(lt * 128, 128), 128)
        wq_v[q] = pin.after(pack(wr_v[0:DF - 1, lanes], wi_v[0:DF - 1, lanes]))
        nyq = pack(wr_v[DF - 1:DF, lanes], wi_v[DF - 1:DF, lanes])
        first = jax.lax.broadcasted_iota(jnp.int32, (64, 128), 0) == 0
        tail = jnp.where(first, jnp.broadcast_to(nyq, (64, 128)), jnp.uint32(0))
        for t, (k0, k1) in enumerate(((1, 4), (2, 3), (0, None))):
            lo = wq_v[q, pl.ds(k0, 64, stride=5), :]
            hi = tail if k1 is None else wq_v[q, pl.ds(k1, 64, stride=5), :]
            w = jnp.concatenate([lo, hi], axis=0).T
            wp_v[t, lanes, :] = w
        return w

    x_copy(0).wait()
    batches = [[c_dfwd, g_copies[1], u_copies[1], x_copy(1)], [x_copy(2), x_copy(3)],
               [x_copy(n) for n in range(4, NT)], [c_wr, c_wi]]
    for c in batches[0]:
        c.start()
    for m in range(4):
        store_xn(0, m, layernorm(0, m, Pin(0)))
    g_copies[0].wait()
    u_copies[0].wait()

    def phase_a(i, with_filter):
        if i in (1, 2):
            for c in batches[i]:
                c.wait()
            for c in batches[i + 1]:
                c.start()
        rows = tile(i)
        pin = Pin(zero)
        gu = _chain(gate_up_steps(ptile(i), 0, pin), gate_up_steps(ptile(i), 1, pin))
        nxt = i + 1
        xn_next, ys = [], []

        def norm(m):
            xn_next.append(layernorm(nxt, m, pin))
            pin.due(xn_next[-1][4], LN_LAG)

        def five_point(h):
            half = pl.ds(_mult(i * (TM // 2) + h * (TM // 4), TM // 4), TM // 4)
            x0, x1, x2, x3, x4 = [pltpu.bitcast(pin.after(xn_v[j, half, :]), bf16).astype(f32) for j in range(5)]
            t1, t2, t3, t4 = x1 + x4, x2 + x3, x1 - x4, x2 - x3
            ys.append([jnp.concatenate([x0 + C1 * t1 + C2 * t2, -S1 * t3 - S2 * t4], axis=1).astype(bf16),
                       jnp.concatenate([x0 + C2 * t1 + C1 * t2, S1 * t4 - S2 * t3], axis=1).astype(bf16),
                       (x0 + t1 + t2).astype(bf16)])

        def dft(t):
            y = jnp.concatenate([ys[0][t], ys[1][t]], axis=0)
            z = _dot(y, pltpu.bitcast(dfwd_v[128 * t:min(128 * (t + 1), D // 2), :], bf16))
            z_v[rows, 256 * t:256 * (t + 1)] = radix4(z, -1)

        first_norm, dft_at = (5, (5, 6, 8)) if i == 0 else (2, DFT_AT)
        for k in range(10):
            if i == 0 and k == 5:
                for c in batches[0]:
                    c.wait()
                for c in batches[1]:
                    c.start()
            next(gu)
            if k < 2:
                five_point(k)
            elif 0 <= k - first_norm < 4 and nxt < NT:
                norm(k - first_norm)
            if with_filter and 5 <= k < 9:
                pin.due(filt(k - 5, (i - NT // 2) * 4 + k - 5, pin), 2)
            if k in dft_at:
                dft(dft_at.index(k))
        for m in range(len(xn_next)):
            store_xn(nxt, m, xn_next[m])

    zero = tw_ref[1, 0].astype(jnp.int32)
    for i in range(NT // 2):
        phase_a(i, False)
    c_wr.wait()
    c_wi.wait()
    later = [c_sf, c_si] + [c[j] for j in range(2, NC) for c in (g_copies, u_copies)]
    for c in later:
        c.start()
    for i in range(NT // 2, NT):
        phase_a(i, True)

    for c in later:
        c.wait()
    for c in (c_wd, c_dinv, c_dinvc):
        c.start()

    def phase_b(c0, carry):
        pin = Pin(c0)
        base = _mult(c0 * NB, NB)

        def twiddle(a0, v, sign):
            if a0 == 0:
                return v
            c, s = tw_ref[0, c0 * 8 + a0], sign * tw_ref[1, c0 * 8 + a0]
            return v[0] * c - v[1] * s, v[0] * s + v[1] * c

        def fft(t):
            for r in range(0, NB, 8):
                def load(a0):
                    rr = pl.ds(a0 * TM + base + r, 8)
                    return twiddle(a0, (pin.after(z_v[rr, 256 * t:256 * t + 128]),
                                        pin.after(z_v[rr, 256 * t + 128:256 * t + 256])), -1)

                def store(c1, v):
                    t_v[t, c1, r:r + 8, :] = v[0]
                    t_v[t, c1, NB + r:NB + r + 8, :] = v[1]
                yield from _fft(load, list(range(8)), -1, store)

        def ifft(t):
            for r in range(0, NB, 8):
                def load(c1):
                    return pin.after(u_v[t, c1, r:r + 8, :]), pin.after(u_v[t, c1, NB + r:NB + r + 8, :])

                def store(a0, v):
                    rr = pl.ds(a0 * TM + base + r, 8)
                    v = twiddle(a0, v, 1)
                    z_v[rr, 256 * t:256 * t + 128] = v[0]
                    z_v[rr, 256 * t + 128:256 * t + 256] = v[1]
                yield from _fft(load, list(range(8)), 1, store)

        def forward(t, c1):
            c = c0 + 4 * c1
            xf = _dot(pltpu.bitcast(sf_v[c], bf16), t_v[t, c1].astype(bf16))
            w = wp_v[t, pl.ds(c, NB, stride=NA), :]
            wr = pltpu.bitcast(w & jnp.uint32(0xFFFF0000), f32)
            wi = pltpu.bitcast(w << 16, f32)
            xr, xi = xf[:NB], xf[NB:]
            return jnp.concatenate([xr * wr - xi * wi, xr * wi + xi * wr], axis=0).astype(bf16)

        def spectral(t):
            for h in range(0, 8, 4):
                ys = [forward(t, c1) for c1 in range(h, h + 4)]
                yield
                for c1 in range(h, h + 4):
                    u_v[t, c1] = _dot(pltpu.bitcast(si_v[c0 + 4 * c1], bf16), ys[c1 - h])
                yield

        gu = _chain(*[gate_up_steps(ptile(2 * c0 + n), j, pin) for n in range(2) for j in range(2, NC)])

        def mixed(t):
            for _ in spectral(t):
                yield
                next(gu)
                yield

        def take(n):
            for _ in range(n):
                next(gu)
                yield

        _interleave(take(7), 7, fft(0), 96)
        _interleave(mixed(0), 8, fft(1), 96)
        _interleave(mixed(1), 8, fft(2), 96)
        _interleave(mixed(2), 8, ifft(0), 96)
        _interleave(take(10), 10, ifft(1), 96)
        _interleave(take(10), 10, ifft(2), 96)
        next(gu)
        return carry

    jax.lax.fori_loop(0, 4, phase_b, 0)

    for c in (c_wd, c_dinv, c_dinvc):
        c.wait()

    def phase_c(i, carry):
        rows = tile(i)
        p1 = _dot(radix4(z_v[rows, 0:256], 1).astype(bf16), pltpu.bitcast(dinv_v[0:128, :], bf16))
        p2 = _dot(radix4(z_v[rows, 256:512], 1).astype(bf16), pltpu.bitcast(dinv_v[128:256, :], bf16))
        p0 = _dot(radix4(z_v[rows, 512:768], 1).astype(bf16), pltpu.bitcast(dinvc_v[...], bf16))
        p1r, p1i, p2r, p2i = p1[:, :128], p1[:, 128:], p2[:, :128], p2[:, 128:]
        a1 = p0 + C1 * p1r + C2 * p2r
        a2 = p0 + C2 * p1r + C1 * p2r
        b1 = S1 * p1i + S2 * p2i
        b2 = S2 * p1i - S1 * p2i
        s = [p0 + p1r + p2r, a1 - b1, a2 - b2, a2 + b2, a1 + b1]
        for n in range(D // 128):
            cn = slice(128 * n, 128 * (n + 1))
            f = _dot(wide(h_v, range(12), ptile(i)), wide(wd_v, [n]))
            y = x_v[i, :, :, cn].reshape(TM, 128).astype(f32) + _silu_times(f, s[n])
            o_v[i, :, :, cn] = y.astype(bf16).reshape(4, NB, 128)
        o_copy(i).start()
        return carry

    jax.lax.fori_loop(0, NT, phase_c, 0, unroll=UNROLL)
    for i in range(NT):
        o_copy(i).wait()


@jax.jit
def pallas_recurrent_scan__spectral_gfnet__swiglu_ffn__prompt_kernel(
    A_x: jax.Array,
    A_w_r: jax.Array,
    A_w_i: jax.Array,
    B_x: jax.Array,
    B_w_gate: jax.Array,
    B_w_up: jax.Array,
    B_w_down: jax.Array,
):
    del B_x
    tw, consts = _constants()
    bf16, f32 = jnp.bfloat16, jnp.float32
    vm = pltpu.VMEM
    out = pl.pallas_call(
        _kernel,
        out_shape=jax.ShapeDtypeStruct((4, NT, NB, D), bf16),
        in_specs=[pl.BlockSpec(memory_space=pltpu.SMEM)] + [pl.BlockSpec(memory_space=pltpu.HBM)] * 11,
        out_specs=pl.BlockSpec(memory_space=pltpu.HBM),
        scratch_shapes=[
            vm((NT, 4, NB, D), bf16), vm((DF, S), bf16), vm((DF, S), bf16),
            vm((12, D // 2, 128), jnp.uint32), vm((12, D // 2, 128), jnp.uint32), vm((5, F // 2, 128), jnp.uint32),
            vm((320, 256), jnp.uint32), vm((256, 256), jnp.uint32), vm((128, 128), jnp.uint32),
            vm((NA, 64, 128), jnp.uint32), vm((NA, 64, 128), jnp.uint32),
            vm((5, S // 2, 128), jnp.uint32), vm((12, S // 2, 128), jnp.uint32), vm((S, 768), f32), vm((3, 8, 128, 128), f32), vm((3, 8, 128, 128), f32),
            vm((4, DF - 1, 128), jnp.uint32), vm((3, S, 128), jnp.uint32), vm((NT, 4, NB, D), bf16),
            pltpu.SemaphoreType.DMA((NT,)), pltpu.SemaphoreType.DMA((36,)), pltpu.SemaphoreType.DMA((NT,)),
        ],
        compiler_params=pltpu.CompilerParams(vmem_limit_bytes=100 * 1024 * 1024),
    )(tw, A_x.reshape(4, NT, NB, D), A_w_r.T, A_w_i.T, B_w_gate, B_w_up, B_w_down, *consts)
    return out.reshape(1, S, D)
```

```python
import math

import numpy as np
import jax
import jax.numpy as jnp
import jax.experimental.pallas as pl
import jax.experimental.pallas.tpu as pltpu

S, D, F = 2048, 640, 1536
DF = D // 2 + 1
TM = 256
NT = S // TM
NC = 6
A_CHUNKS = 2
FC = F // NC
NA, NB = 32, 64
EPS = 1e-5


def _constants():
    lane = np.arange(128)
    ka = np.where(lane < 64, 1 + 5 * lane, 4 + 5 * (lane - 64))
    kb = np.where(lane < 64, 2 + 5 * lane, 3 + 5 * (lane - 64))
    n2 = np.arange(128)[:, None]
    sig = np.where(np.arange(128) < 64, 1.0, -1.0)[None, :]

    def three(k):
        th = 2 * np.pi * ((n2 * k[None, :]) % D) / D
        c, s = np.cos(th), sig * np.sin(th)
        return [c, -s - c, c - s], [m.T * (2.0 / D) for m in (c, s - c, c + s)]

    (fa, ia), (fb, ib) = three(ka), three(kb)
    kp = 5 * np.where(lane <= 64, lane, lane - 64)
    th = 2 * np.pi * ((n2 * kp[None, :]) % D) / D
    fc = np.where(lane[None, :] <= 64, np.cos(th), -np.sin(th))
    alpha = np.where((kp == 0) | (kp == D // 2), 1.0, 2.0)[:, None]
    dfwd, dinv = np.stack(fa + fb), np.stack(ia + ib)
    dinvc = np.concatenate([fc, fc.T * alpha / D], axis=0)

    b = np.arange(NB)[None, None, :]
    d = np.arange(NB)[None, :, None]
    c = np.arange(NA)[:, None, None]
    ph = 2 * np.pi * ((b * (c + NA * d)) % S) / S
    mr, mi = np.cos(ph), -np.sin(ph)
    sf = np.concatenate([np.concatenate([mr, -mi], axis=2),
                         np.concatenate([mi, mr], axis=2)], axis=1)
    si = np.transpose(sf, (0, 2, 1)) / S

    bf = jnp.bfloat16

    def pairs(a):
        u = a.astype(bf).view(np.uint16).astype(np.uint32)
        return u[..., 0::2, :] | (u[..., 1::2, :] << 16)

    return tuple(pairs(a) for a in (dfwd, dinv, dinvc, sf, si))


def _cmul_const(z, k, n, sign):
    re, im = z
    k = k % n
    if k == 0:
        return z
    if 2 * k == n:
        return -re, -im
    if 4 * k == n:
        return (-im, re) if sign > 0 else (im, -re)
    c = math.cos(2 * math.pi * k / n)
    s = sign * math.sin(2 * math.pi * k / n)
    if 8 * k == n:
        return ((re - im) * c, (re + im) * c) if sign > 0 else ((re + im) * c, (im - re) * c)
    if 8 * k == 3 * n:
        return ((re + im) * c, (im - re) * c) if sign > 0 else ((re - im) * c, (re + im) * c)
    return (re * c - im * s, re * s + im * c)


def _fft(load, idx, sign, store=None):
    n = len(idx)
    if n == 1:
        return [load(idx[0])]
    ev = yield from _fft(load, idx[0::2], sign)
    od = yield from _fft(load, idx[1::2], sign)
    out = [None] * n
    for k in range(n // 2):
        er, ei = ev[k]
        if 4 * k == n:
            orr, oi = od[k]
            if sign > 0:
                out[k], out[k + n // 2] = (er - oi, ei + orr), (er + oi, ei - orr)
            else:
                out[k], out[k + n // 2] = (er + oi, ei - orr), (er - oi, ei + orr)
        else:
            tr, ti = _cmul_const(od[k], k, n, sign)
            out[k], out[k + n // 2] = (er + tr, ei + ti), (er - tr, ei - ti)
        if store is not None:
            store(k, out[k])
            store(k + n // 2, out[k + n // 2])
        yield
    return out


def _chain(*gens):
    for g in gens:
        yield from g


def _a_plan():
    def chunk(i, j, extra):
        return [e for k in range(5) for e in [("g", i, j)] + extra.get(k, [])]

    def norms(i, ms):
        return [("norm", i, m) for m in ms] if i < NT else []

    plan = [("five", 0, 0), ("five", 0, 1), ("dft", 0, 0), ("dft", 0, 1), ("dft", 0, 2), ("arrive", 0, 5)]
    plan += chunk(0, 0, {1: [("arrive", 0, 0)] + norms(1, (0, 1)), 2: norms(1, (2, 3))})
    plan += chunk(1, 0, {0: [("five", 1, 0)], 1: [("five", 1, 1)], 3: [("dft", 1, 0), ("dft", 1, 1), ("dft", 1, 2)]})
    plan += [("arrive", 0, 1)]
    plan += chunk(0, 1, {3: [("arrive", 0, 2)] + norms(2, [0])})
    plan += chunk(1, 1, {0: norms(2, [1]), 1: norms(2, [2]), 2: norms(2, [3])})
    for i in range(2, NT):
        extra = {k: [] for k in range(10)}
        if i == 4:
            extra[1].append(("arrive", 0, 3))
        for h in range(2):
            extra[h].append(("five", i, h))
        for m in range(4):
            extra[2 + 2 * m] += norms(i + 1, [m])
            if i >= 4:
                extra[3 + 2 * m].append(("filt", 0, 4 * (i - 4) + m))
        for t in range(3):
            extra[(3, 7, 7)[t]].append(("dft", i, t))
        plan += [("reset", i, 0)] + chunk(i, 0, extra) + chunk(i, 1, {k - 5: v for k, v in extra.items()})
    at = [n for n, e in enumerate(plan) if e == ("g", NT - 1, 0)]
    plan.insert(at[4] + 1, ("xsum", 0, 1))
    plan.insert(at[3] + 1, ("xsum", 0, 0))
    at = [n for n, e in enumerate(plan) if e == ("g", NT - 1, 1)]
    plan.insert(at[3] + 1, ("wsum", 0, 2 * A_CHUNKS))
    plan.insert(at[3] + 1, ("arrive", 0, 4))
    return plan


def _b_plan():
    g = "g"

    def spread(n, total, idle):
        m = n - idle
        return [(g, total * (k + 1) // m - total * k // m) for k in range(m)] + [(g, 0)] * idle
    plan = spread(11, 96, 2)
    for t in range(3):
        steps = iter(spread(8, 96 if t < 2 else 0, 1))
        for ch in "agggAgbgggBg":
            plan.append(next(steps) if ch == "g" else (("f" if ch in "ab" else "i", t, int(ch in "bB")), 0))
        if t == 1:
            plan += spread(13, 96, 0)
    return plan + spread(24, 192, 1)


A_PLAN, B_PLAN = _a_plan(), _b_plan()
C1, C2 = math.cos(2 * math.pi / 5), math.cos(4 * math.pi / 5)
S1, S2 = math.sin(2 * math.pi / 5), math.sin(4 * math.pi / 5)


def _dot(a, b):
    return jnp.dot(a, b, preferred_element_type=jnp.float32)


def _silu_times(v, u):
    hv = 0.5 * v
    a = hv * u
    return a + a * jnp.tanh(hv)


def _kernel(one_hbm, x_hbm, wr_hbm, wi_hbm, wg_hbm, wu_hbm, wd_hbm,
            dfwd_hbm, dinv_hbm, dinvc_hbm, sf_hbm, si_hbm,
            o_hbm,
            x_v, wr_v, wi_v, wg_v, wu_v, wd_v, dfwd_v, dinv_v, dinvc_v, sf_v, si_v,
            xn_v, h_v, z_v, t_v, u_v, wq_v, wp_v, o_v, xs_v, ws_v, hs_v, wds_v, one_v, sem_x, sem_w, sem_o):
    f32, bf16 = jnp.float32, jnp.bfloat16

    def x_copy(i):
        return pltpu.make_async_copy(x_hbm.at[:, i], x_v.at[i], sem_x.at[i])

    def col_copy(src, dst, lo, hi, sem):
        cols = pl.ds(lo, hi - lo)
        return pltpu.make_async_copy(src.at[:, cols], dst.at[:, cols], sem_w.at[sem])

    def wide(w, slabs, rows):
        return pltpu.bitcast(jnp.concatenate([w[n, rows, :] for n in slabs], axis=1), bf16)

    def o_copy(i, part):
        cols = (pl.ds(0, 512), pl.ds(512, 128), pl.ds(0, D))[part]
        return pltpu.make_async_copy(o_v.at[i, :, :, cols], o_hbm.at[:, i, :, cols], sem_o.at[2 * i + part % 2])

    spans = ((0, FC), (FC, 2 * FC), (2 * FC, F))
    g_copies = [col_copy(wg_hbm, wg_v, lo, hi, j) for j, (lo, hi) in enumerate(spans)]
    u_copies = [col_copy(wu_hbm, wu_v, lo, hi, 3 + j) for j, (lo, hi) in enumerate(spans)]
    whole = [pltpu.make_async_copy(s_, d_, sem_w.at[6 + n]) for n, (s_, d_) in enumerate([
        (dfwd_hbm, dfwd_v), (wr_hbm, wr_v), (wi_hbm, wi_v), (sf_hbm, sf_v),
        (si_hbm, si_v), (wd_hbm, wd_v), (one_hbm, one_v), (dinv_hbm, dinv_v), (dinvc_hbm, dinvc_v)])]
    c_dfwd, c_wr, c_wi, c_sf, c_si, c_wd, c_one, c_dinv, c_dinvc = whole

    for c in (x_copy(0), c_one, c_dfwd, c_dinvc):
        c.start()
    for c in (g_copies[0], u_copies[0]):
        c.start(priority=1)

    class Pairs:
        def __init__(self, ref):
            self.ref = ref

        def __getitem__(self, idx):
            n, rows, _ = idx
            return pltpu.bitcast(self.ref[2 * rows.start:2 * rows.stop, 128 * n:128 * (n + 1)], jnp.uint32)

    wg_v, wu_v, wd_v = Pairs(wg_v), Pairs(wu_v), Pairs(wd_v)

    def tile(i):
        return pl.ds(i * TM, TM)

    def ptile(i):
        return pl.ds(i * (TM // 2), TM // 2)

    class Pin:
        def __init__(self):
            self.keep = one_v[...] > 0
            self.dep = None
            self.queue = [[] for _ in range(5)]

        def mark(self, v):
            self.dep = v[0:8, 0:128]

        def after(self, v):
            if self.dep is None:
                return v
            n = v.shape[0] // 8
            dep = self.dep if v.dtype == f32 else pltpu.bitcast(self.dep, v.dtype)
            return jnp.where(jnp.concatenate([self.keep] * n, axis=0), v, jnp.concatenate([dep] * n, axis=0))

        def due(self, d, lag):
            self.queue[lag].append(d if d.dtype == jnp.uint32 else pltpu.bitcast(d, jnp.uint32))

        def lhs(self, slabs, rows, src=xn_v):
            parts = [src[n, rows, :] for n in slabs]
            for n, d in enumerate(self.queue[0]):
                v, r = parts[n % len(parts)], d.shape[0]
                head = jnp.where(jnp.concatenate([self.keep] * (r // 8), axis=0), v[:r], d)
                parts[n % len(parts)] = head if r == v.shape[0] else jnp.concatenate([head, v[r:]], axis=0)
            self.queue = self.queue[1:] + [[]]
            return pltpu.bitcast(jnp.concatenate(parts, axis=1), bf16)

    def gate_up_steps(rows, j, pin):
        xt = pin.lhs([4], rows)
        pair = (2 * j, 2 * j + 1)
        gt, ut = _dot(xt, wide(wg_v, pair, slice(256, D // 2))), _dot(xt, wide(wu_v, pair, slice(256, D // 2)))
        pin.mark(gt)
        yield
        for n in range(2):
            g = _dot(pin.lhs(range(4), rows), wide(wg_v, [pair[n]], slice(0, 256)))
            pin.mark(g)
            g = g + gt[:, 128 * n:128 * (n + 1)]
            yield
            u = _dot(pin.lhs(range(4), rows), wide(wu_v, [pair[n]], slice(0, 256)))
            pin.mark(u)
            h_v[pair[n], rows, :] = pltpu.bitcast(
                _silu_times(g, u + ut[:, 128 * n:128 * (n + 1)]).astype(bf16), jnp.uint32)
            yield

    def strassen_steps(p, n, pin):
        ra, rb = ptile(2 * p), ptile(2 * p + 1)
        lo, hi, tail = slice(0, 128), slice(128, 256), slice(256, D // 2)
        gate = {}

        def prod(src, slabs, rows, w):
            m = _dot(pin.lhs(slabs, rows, src), pltpu.bitcast(w, bf16))
            pin.mark(m)
            return m

        for e, w in enumerate((wg_v, wu_v)):
            def emit(t, k, y):
                if e == 0:
                    gate[t, k] = y
                else:
                    h = _silu_times(gate[t, k], y).astype(bf16)
                    h_v[n + k, ptile(2 * p + t), :] = pltpu.bitcast(h, jnp.uint32)

            ws = ws_v.at[n + e - 2 * A_CHUNKS]

            def with_tail(slabs, rows, wsum_, k):
                x = jnp.concatenate([pin.lhs(slabs, ptile(p), xs_v), pltpu.bitcast(xn_v[4, rows, :], bf16)], axis=1)
                m = _dot(x, pltpu.bitcast(jnp.concatenate([wsum_, w[n + k, tail, :]], axis=0), bf16))
                pin.mark(m)
                return m

            m1 = prod(xs_v, (0, 1), ptile(p), ws[0])
            yield
            m4 = prod(xn_v, (2, 3), rb, ws[2])
            ya = m1 + m4
            yield
            ya = ya + with_tail((8, 9), ra, ws[4], 0)
            yield
            m5 = prod(xs_v, (4, 5), ptile(p), w[n + 1, hi, :])
            emit(0, 0, ya - m5)
            yield
            m3 = prod(xn_v, (0, 1), ra, ws[1])
            yb = m1 + m3
            yield
            emit(0, 1, m5 + m3 + prod(xn_v, (4,), ra, w[n + 1, tail, :]))
            yield
            m2 = prod(xs_v, (2, 3), ptile(p), w[n, lo, :])
            yb = yb - m2
            yield
            emit(1, 0, m4 + m2 + prod(xn_v, (4,), rb, w[n, tail, :]))
            yield
            emit(1, 1, yb + with_tail((6, 7), rb, ws[3], 1))
            yield

    def wsum(n, pin):
        w11, w21, w12, w22 = [pltpu.bitcast(pin.after((wg_v, wu_v)[n % 2][e, r:r + 128, :]), bf16).astype(f32)
                              for e in (n & ~1, n | 1) for r in (0, 128)]
        for e, v in enumerate((w11 + w22, w12 - w22, w21 - w11, w11 + w12, w21 + w22)):
            v = pltpu.bitcast(v.astype(bf16), jnp.uint32)
            ws_v[n - 2 * A_CHUNKS, e] = v
        pin.due(v, 3)

    def xsum(p, k, pin):
        q = TM // 4
        for e in range(2):
            a_lo, a_hi, b_lo, b_hi = [
                pltpu.bitcast(pin.after(xn_v[j + e, pl.ds(t * (TM // 2) + k * q, q), :]), bf16).astype(f32)
                for t in (2 * p, 2 * p + 1) for j in (0, 2)]
            for n, v in enumerate((a_lo + b_hi, b_lo + b_hi, a_lo + a_hi, b_lo - a_lo, a_hi - b_hi)):
                v = pltpu.bitcast(v.astype(bf16), jnp.uint32)
                xs_v[2 * n + e, pl.ds(p * (TM // 2) + k * q, q), :] = v
            pin.due(v, 3)

    def dsum(n, r, pin):
        w11, w21, w12, w22 = [pltpu.bitcast(pin.after(wd_v[e, o + r:o + r + 128, :]), bf16).astype(f32)
                              for e in (n, n + 2) for o in (0, F // 4)]
        for e, v in enumerate((w11 + w22, w12 - w22, w21 - w11, w11 + w12, w21 + w22)):
            v = pltpu.bitcast(v.astype(bf16), jnp.uint32)
            wds_v[n, e, r:r + 128, :] = v
        pin.due(v, 3)

    def hsum(p, e, pin):
        a_lo, a_hi, b_lo, b_hi = [pltpu.bitcast(pin.after(h_v[j + e, ptile(t), :]), bf16).astype(f32)
                                  for t in (2 * p, 2 * p + 1) for j in (0, 6)]
        for n, v in enumerate((a_lo + b_hi, b_lo + b_hi, a_lo + a_hi, b_lo - a_lo, a_hi - b_hi)):
            v = pltpu.bitcast(v.astype(bf16), jnp.uint32)
            hs_v[6 * n + e, ptile(p % 2), :] = v
        pin.due(v, 1 if p else 3)

    def pack(re, im):
        return (pltpu.bitcast(re.astype(f32), jnp.uint32)
                | (pltpu.bitcast(im.astype(f32), jnp.uint32) >> 16))

    def layernorm(i, m, pin):
        x = jnp.concatenate(
            [pltpu.bitcast(pin.after(pltpu.bitcast(x_v[i, m, :, 128 * n:128 * (n + 1)], jnp.uint32)), bf16)
             for n in range(5)], axis=1).astype(f32)
        xc = x - jnp.mean(x, axis=-1, keepdims=True)
        v = jnp.mean(xc * xc, axis=-1, keepdims=True)
        xn = pltpu.bitcast((xc * jax.lax.rsqrt(v + EPS)).astype(bf16), jnp.uint32)
        return [xn[:, 128 * n:128 * (n + 1)] for n in range(5)]

    def store_xn(i, m, slabs):
        rows = pl.ds(i * (TM // 2) + m * (NB // 2), NB // 2)
        for n in range(5):
            xn_v[n, rows, :] = slabs[n]

    def radix4(v, sign):
        re = [v[NB * m:NB * (m + 1), :128] for m in range(4)]
        im = [v[NB * m:NB * (m + 1), 128:] for m in range(4)]
        ar, ai, br, bi = re[0] + re[2], im[0] + im[2], re[0] - re[2], im[0] - im[2]
        cr, ci, dr, di = re[1] + re[3], im[1] + im[3], re[1] - re[3], im[1] - im[3]
        lo, hi = (br + di, bi - dr), (br - di, bi + dr)
        out = [(ar + cr, ai + ci), lo if sign < 0 else hi, (ar - cr, ai - ci), hi if sign < 0 else lo]
        return jnp.concatenate([jnp.concatenate(o, axis=1) for o in out], axis=0)

    def cdot(ys, mats, t):
        k1, k2, k3 = [_dot(y, pltpu.bitcast(mats[3 * t + n], bf16)) for n, y in enumerate(ys)]
        return k1 - k3, k1 + k2

    def conj_upper(im):
        return im * jnp.where(jax.lax.broadcasted_iota(jnp.int32, (1, 128), 1) < 64, 1.0, -1.0)

    def filt(q, lt, pin):
        lanes = pl.ds(lt * 128, 128)
        wq_v[q, 0:DF - 1, :] = pack(wr_v[0:DF - 1, lanes], wi_v[0:DF - 1, lanes])
        nyq = pack(wr_v[DF - 1:DF, lanes], wi_v[DF - 1:DF, lanes])
        first = jax.lax.broadcasted_iota(jnp.int32, (64, 128), 0) == 0
        tail = jnp.where(first, jnp.broadcast_to(nyq, (64, 128)), jnp.uint32(0))
        for t, (k0, k1) in enumerate(((1, 4), (2, 3), (0, None))):
            lo = wq_v[q, pl.ds(k0, 64, stride=5), :]
            hi = tail if k1 is None else wq_v[q, pl.ds(k1, 64, stride=5), :]
            w = jnp.concatenate([lo, hi], axis=0).T
            for e in range(128 // NA):
                wp_v[t, pl.ds((lt * (128 // NA) + e) * (NA + 1), NA), :] = w[NA * e:NA * (e + 1)]
        return w

    for c in (x_copy(0), c_one, c_dfwd, c_dinvc):
        c.wait()
    batches = [[x_copy(1)], [g_copies[1], u_copies[1]], [x_copy(n) for n in range(2, 5)],
               [x_copy(5), x_copy(6), x_copy(7), c_wr, c_wi],
               [c_sf, c_si, g_copies[2], u_copies[2]], [g_copies[0], u_copies[0]]]
    x_copy(1).start(priority=1)
    for m in range(4):
        store_xn(0, m, layernorm(0, m, Pin()))

    pin = Pin()
    steps, five = {}, {}
    for op, i, k in A_PLAN:
        if op == "g":
            if (i, k) not in steps:
                steps[i, k] = gate_up_steps(ptile(i), k, pin)
            next(steps[i, k])
        elif op == "arrive":
            for c in batches[k]:
                c.wait()
            for c in {5: batches[1], 0: batches[2], 1: batches[3], 3: batches[4]}.get(k, []):
                c.start(priority=1)
        elif op == "reset":
            pin.dep, pin.queue = None, [[] for _ in pin.queue]
        elif op == "norm":
            slabs = layernorm(i, k, pin)
            store_xn(i, k, slabs)
            pin.due(slabs[4], 1)
        elif op == "filt":
            pin.due(filt(k % 4, k, pin), 2)
        elif op == "wsum":
            wsum(k, pin)
        elif op == "xsum":
            xsum(i, k, pin)
        elif op == "five":
            half = pl.ds(i * (TM // 2) + k * (TM // 4), TM // 4)
            x0, x1, x2, x3, x4 = [pltpu.bitcast(pin.after(xn_v[j, half, :]), bf16).astype(f32) for j in range(5)]
            t1, t2, t3, t4 = x1 + x4, x2 + x3, x1 - x4, x2 - x3
            y1r, y1i = x0 + C1 * t1 + C2 * t2, -S1 * t3 - S2 * t4
            y2r, y2i = x0 + C2 * t1 + C1 * t2, S1 * t4 - S2 * t3
            five[i, k] = [v.astype(bf16) for v in (y1r + y1i, y1r, y1i, y2r + y2i, y2r, y2i, x0 + t1 + t2)]
        else:
            ys = [jnp.concatenate([five[i, 0][n], five[i, 1][n]], axis=0) for n in range(3 * k, min(3 * k + 3, 7))]
            if k < 2:
                re, im = cdot(ys, dfwd_v, k)
                z = jnp.concatenate([re, conj_upper(im)], axis=1)
            else:
                z = _dot(ys[0], pltpu.bitcast(dinvc_v[0:64, :], bf16))
                lane = jax.lax.broadcasted_iota(jnp.int32, z.shape, 1)
                z = jnp.concatenate([z, jnp.where(lane % 64 == 0, 0.0, pltpu.roll(z, 64, 1))], axis=1)
            z_v[tile(i), 256 * k:256 * (k + 1)] = radix4(z, -1)

    for c in (c_wd, c_dinv):
        c.start()

    def phase_b(c0):
        base = c0 * NB
        last = []

        def twiddle(a0, v, sign):
            return _cmul_const(v, a0 * c0, NA, sign)

        def fft(t):
            for r in range(0, NB, 8):
                def load(a0):
                    rr = pl.ds(a0 * TM + base + r, 8)
                    return twiddle(a0, (pin.after(z_v[rr, 256 * t:256 * t + 128]),
                                        pin.after(z_v[rr, 256 * t + 128:256 * t + 256])), -1)

                def store(c1, v):
                    t_v[t, c1, r:r + 8, :] = v[0]
                    t_v[t, c1, NB + r:NB + r + 8, :] = v[1]
                    last.append(v[1])
                yield from _fft(load, list(range(8)), -1, store)

        def ifft(t):
            for r in range(0, NB, 8):
                def load(c1):
                    return pin.after(u_v[t, c1, r:r + 8, :]), pin.after(u_v[t, c1, NB + r:NB + r + 8, :])

                def store(a0, v):
                    rr = pl.ds(a0 * TM + base + r, 8)
                    v = twiddle(a0, v, 1)
                    z_v[rr, 256 * t:256 * t + 128] = v[0]
                    z_v[rr, 256 * t + 128:256 * t + 256] = v[1]
                    last.append(v[1])
                yield from _fft(load, list(range(8)), 1, store)

        def forward(t, c1):
            c = c0 + 4 * c1
            xf = _dot(pltpu.bitcast(sf_v[c], bf16), t_v[t, c1].astype(bf16))
            w = wp_v[t, pl.ds(c, NB, stride=NA + 1), :]
            wr = pltpu.bitcast(w & jnp.uint32(0xFFFF0000), f32)
            wi = pltpu.bitcast(w << 16, f32)
            xr, xi = xf[:NB], xf[NB:]
            return jnp.concatenate([xr * wr - xi * wi, xr * wi + xi * wr], axis=0).astype(bf16)

        gu = _chain(*[strassen_steps(c0, n, pin) for n in range(2 * A_CHUNKS, 2 * NC, 2)])
        vpu = _chain(fft(0), fft(1), fft(2), ifft(0), ifft(1), ifft(2))
        ys = {}
        done = 0
        for slot, quota in B_PLAN:
            if slot == "g":
                next(gu)
                done += 1
                slab, k = 2 * A_CHUNKS + done // 9, done % 9
                if c0 == 0 and k == 1 and slab + 1 < 2 * NC:
                    wsum(slab + 1, pin)
                if c0 == 1 and done == 1:
                    for c in (c_wd, c_dinv):
                        c.wait()
                if c0 == 1 and k == 2 and slab < 2 * A_CHUNKS + 6:
                    dsum((slab - 2 * A_CHUNKS) // 3, 128 * ((slab - 2 * A_CHUNKS) % 3), pin)
                if c0 == 2 and k == 2 and slab < 2 * A_CHUNKS + 6:
                    hsum(0, slab - 2 * A_CHUNKS, pin)
                if c0 < 3 and k == 6 and slab >= 2 * NC - 2:
                    xsum(c0 + 1, slab - (2 * NC - 2), pin)
            else:
                t, h = slot[1:]
                for c1 in range(4 * h, 4 * h + 4):
                    if slot[0] == "f":
                        ys[t, c1] = forward(t, c1)
                    else:
                        u_v[t, c1] = _dot(pltpu.bitcast(si_v[c0 + 4 * c1], bf16), ys.pop((t, c1)))
            for _ in range(quota):
                next(vpu)
            if last and slot == "g":
                pin.due(jnp.concatenate(last[-16:], axis=0), 3)
                last.clear()

    for c0 in range(4):
        phase_b(c0)

    ready = {}

    def phase_c(p):
        ta, tb = 2 * p, 2 * p + 1
        ra, rb, rp = ptile(ta), ptile(tb), ptile(p % 2)
        lo, hi = slice(0, F // 4), slice(F // 4, F // 2)
        spec = {}

        def prod(src, slabs, rows, w):
            m = _dot(pin.lhs(slabs, rows, src), pltpu.bitcast(w, bf16))
            pin.mark(m)
            return m

        def prep(i, t):
            z = jnp.concatenate([pin.after(z_v[tile(i), 256 * t + e:256 * t + e + 128]) for e in (0, 128)], axis=1)
            z = radix4(z, 1)
            if t == 2:
                lane = jax.lax.broadcasted_iota(jnp.int32, (TM, 128), 1)
                z = jnp.where(lane <= 64, z[:, :128], pltpu.roll(z[:, 128:], 64, 1))
                ready[i, t] = z.astype(bf16)
            else:
                re, im = z[:, :128], conj_upper(z[:, 128:])
                ready[i, t] = [v.astype(bf16) for v in (re + im, re, im)]

        def idft(i, t):
            z = ready.pop((i, t))
            spec[i, t] = _dot(z, pltpu.bitcast(dinvc_v[64:128, :], bf16)) if t == 2 else cdot(z, dinv_v, t)
            if t == 2:
                p0, (p1r, p1i), (p2r, p2i) = spec[i, 2], spec[i, 0], spec[i, 1]
                a1, a2 = p0 + C1 * p1r + C2 * p2r, p0 + C2 * p1r + C1 * p2r
                b1, b2 = S1 * p1i + S2 * p2i, S2 * p1i - S1 * p2i
                spec[i] = [p0 + p1r + p2r, a1 - b1, a2 - b2, a2 + b2, a1 + b1]

        def finish(i, n, f):
            cn = slice(128 * n, 128 * (n + 1))
            y = x_v[i, :, :, cn].reshape(TM, 128).astype(f32) + _silu_times(f, spec[i][n])
            y = y.astype(bf16)
            o_v[i, :, :, cn] = y.reshape(4, NB, 128)
            pin.due(pltpu.bitcast(y, jnp.uint32), 1)

        units = [(i, t) for i in (ta, tb) for t in range(3)]
        slot = iter(range(14))
        if p == 0:
            prep(*units[0])

        def between():
            k = next(slot)
            if k < 5:
                prep(*units[k + 1])
            if k < 6:
                idft(*units[k])
            if p < 3 and k == 13:
                prep(ta + 2, units[0][1])
            if p < 3 and 7 <= k < 13:
                hsum(p + 1, k - 7, pin)

        for n in range(2):
            def hs(k):
                return range(6 * k, 6 * k + 6)
            m1 = prod(hs_v, hs(0), rp, wds_v[n, 0])
            if n == 0 and p > 0:
                for i in (ta - 2, tb - 2):
                    o_copy(i, 2).start()
            between()
            m4 = prod(h_v, hs(1), rb, wds_v[n, 2])
            fa = m1 + m4
            between()
            fa = fa + prod(hs_v, hs(4), rp, wds_v[n, 4])
            between()
            m5 = prod(hs_v, hs(2), rp, wd_v[n + 2, hi, :])
            between()
            finish(ta, n, fa - m5)
            m3 = prod(h_v, hs(0), ra, wds_v[n, 1])
            finish(ta, n + 2, m5 + m3)
            fb = m1 + m3
            between()
            m2 = prod(hs_v, hs(1), rp, wd_v[n, lo, :])
            between()
            finish(tb, n, m4 + m2)
            fb = fb - m2
            finish(tb, n + 2, fb + prod(hs_v, hs(3), rp, wds_v[n, 3]))
            between()
        f4 = prod(h_v, range(12), ra, wd_v[4, 0:F // 2, :])
        if p == 3:
            o_copy(ta, 0).start()
            o_copy(tb, 0).start()
        finish(ta, 4, f4)
        finish(tb, 4, prod(h_v, range(12), rb, wd_v[4, 0:F // 2, :]))
        if p == 3:
            o_copy(ta, 1).start()
            o_copy(tb, 1).start()

    for p in range(NT // 2):
        phase_c(p)
    for i in range(NT):
        for part in (2,) if i < NT - 2 else (0, 1):
            o_copy(i, part).wait()


@jax.jit
def pallas_recurrent_scan__spectral_gfnet__swiglu_ffn__prompt_kernel(
    A_x: jax.Array,
    A_w_r: jax.Array,
    A_w_i: jax.Array,
    B_x: jax.Array,
    B_w_gate: jax.Array,
    B_w_up: jax.Array,
    B_w_down: jax.Array,
):
    del B_x
    consts = _constants()
    bf16, f32 = jnp.bfloat16, jnp.float32
    vm = pltpu.VMEM
    out = pl.pallas_call(
        _kernel,
        out_shape=jax.ShapeDtypeStruct((4, NT, NB, D), bf16),
        in_specs=[pl.BlockSpec(memory_space=pltpu.HBM)] * 12,
        out_specs=pl.BlockSpec(memory_space=pltpu.HBM),
        scratch_shapes=[
            vm((NT, 4, NB, D), bf16), vm((DF, S), bf16), vm((DF, S), bf16),
            vm((D, F), bf16), vm((D, F), bf16), vm((F, D), bf16),
            vm((6, 64, 128), jnp.uint32), vm((6, 64, 128), jnp.uint32), vm((128, 128), jnp.uint32),
            vm((NA, 64, 128), jnp.uint32), vm((NA, 64, 128), jnp.uint32),
            vm((5, S // 2, 128), jnp.uint32), vm((12, S // 2, 128), jnp.uint32), vm((S, 768), f32), vm((3, 8, 128, 128), f32), vm((3, 8, 128, 128), f32),
            vm((4, DF + 7, 128), jnp.uint32), vm((3, (NB + 1) * (NA + 1) + 7, 128), jnp.uint32), vm((NT, 4, NB, D), bf16),
            vm((10, S // 4, 128), jnp.uint32), vm((2 * (NC - A_CHUNKS), 5, 128, 128), jnp.uint32),
            vm((30, TM, 128), jnp.uint32), vm((2, 5, F // 4, 128), jnp.uint32), vm((8, 128), jnp.int32),
            pltpu.SemaphoreType.DMA((NT,)), pltpu.SemaphoreType.DMA((15,)), pltpu.SemaphoreType.DMA((2 * NT,)),
        ],
        compiler_params=pltpu.CompilerParams(vmem_limit_bytes=100 * 1024 * 1024),
    )(np.arange(1, 1025, dtype=np.int32).reshape(8, 128), A_x.reshape(4, NT, NB, D), A_w_r.T, A_w_i.T, B_w_gate, B_w_up, B_w_down, *consts)
    return out.reshape(1, S, D)
```
